```python
import os as _os
_os.environ.setdefault("JAX_PLATFORMS", "cpu")
import jax
import jax.numpy as jnp

def _softmax(x, axis=-1):
    return jax.nn.softmax(x, axis=axis)
def _gelu(x):
    return jax.nn.gelu(x, approximate=True)
def _silu(x):
    return jax.nn.silu(x)
def _sigmoid(x):
    return jax.nn.sigmoid(x)
def _layernorm(x, axis=-1, eps=1e-5):
    m = jnp.mean(x, axis=axis, keepdims=True)
    v = jnp.var(x, axis=axis, keepdims=True)
    return (x - m) / jnp.sqrt(v + eps)
def _scatter_add(tgt, idx, src, axis=0):
    return tgt.at[idx].add(src)
def _segment_sum(src, seg, n):
    return jax.ops.segment_sum(src, seg, n)
class _Rng:
    def __init__(self, key):
        self._k = key
    def _next(self):
        self._k, sub = jax.random.split(self._k)
        return sub
    def normal(self, shape):
        return jax.random.normal(self._next(), shape, dtype=jnp.bfloat16)
    def randint(self, lo, hi, shape):
        return jax.random.randint(self._next(), shape, lo, hi, dtype=jnp.int32)
    def uniform(self, shape, lo=0.0, hi=1.0):
        return jax.random.uniform(self._next(), shape, jnp.bfloat16, lo, hi)
    def permutation(self, n):
        return jax.random.permutation(self._next(), n)


kernel_name = 'standalone__channel_attn_cbam__vision'

def setup_inputs():
    _rng = _Rng(jax.random.key(int.from_bytes(__import__("os").urandom(4), "little")))
    _w = (lambda a: (lambda t: t.astype(jnp.bfloat16) if jnp.issubdtype(t.dtype, jnp.floating) else t)(jnp.asarray(a)))
    H = W = 224
    C = 192
    r = max(C // 4, 1)
    return {
        "x": _w((lambda *s: _rng.normal(s) * 0.2)(1, H, W, C) + (lambda *s: _rng.normal(s) * 0.2)(1, 1, 1, C) * 2.0),
        "w1": _w((lambda *s: _rng.normal(s) * 0.2)(C, r)),
        "w2": _w((lambda *s: _rng.normal(s) * 0.2)(r, C)),
    }

def reference(x, w1, w2):
    B, H, W, C = x.shape
    xf = x.reshape(B, H * W, C)
    gap = jnp.mean(xf, 1)
    gmp = jnp.amax(xf, 1)
    h_a = gap @ w1
    h_a = h_a * (lambda x, dt: x.astype(dt))(h_a > 0, h_a.dtype)
    h_m = gmp @ w1
    h_m = h_m * (lambda x, dt: x.astype(dt))(h_m > 0, h_m.dtype)
    scale = _sigmoid(h_a @ w2 + h_m @ w2)
    return x * scale[:, None, None, :]
```

```python
import functools
import jax, jax.numpy as jnp
from jax import lax
import jax.experimental.pallas as pl
import jax.experimental.pallas.tpu as pltpu

F32 = jnp.float32
BF16 = jnp.bfloat16

def _rnd(v):
    return v.astype(BF16).astype(F32)

def default_jobs(G, Sh, C):
    jobs = []
    for c0 in range(0, 160, 32):
        jobs.append((c0, 32, 0, G, 0, Sh))
    jobs.append((160, 24, 0, G, 0, Sh))
    jobs.append((184, 8, 0, 5, 0, Sh))
    jobs.append((184, 8, 5, 1, 0, Sh))
    jobs.append((184, 8, 6, 1, 0, 24))
    jobs.append((184, 8, 6, 1, 24, 8))
    return jobs

def make(jobs=None, Sh=32, CB=64, unroll1=4, nocheck=True, split_first=True, skip=()):
    def fn(x, w1, w2):
        B, H, W, C = x.shape
        R = w1.shape[1]
        assert B == 1
        G = H // Sh
        NCB = C // CB
        xt = jnp.transpose(x, (0, 1, 3, 2)).reshape(G, Sh, C, W)
        w1t = jnp.transpose(w1)
        jbs = jobs or default_jobs(G, Sh, C)
        NJ = len(jbs)
        inv_hw = 1.0 / (H * W)

        def kernel(x_hbm, w1t_hbm, w2_hbm, o_hbm, xbuf, w1t_v, w2_v, w1c, w2c, scl, in_sems, w_sem, out_sem):
            def in_copy(i):
                c0, nc, g0, ng, r0, nr = jbs[i]
                sl = (pl.ds(g0, ng), pl.ds(r0, nr), pl.ds(c0, nc))
                return pltpu.make_async_copy(x_hbm.at[sl], xbuf.at[sl], in_sems.at[i])
            wc1 = pltpu.make_async_copy(w1t_hbm, w1t_v, w_sem.at[0])
            wc2 = pltpu.make_async_copy(w2_hbm, w2_v, w_sem.at[1])
            in_copy(0).start(priority=1)
            wc1.start()
            wc2.start()
            for i in range(1, NJ):
                in_copy(i).start(priority=1)
            wc1.wait()
            wc2.wait()
            w1c[...] = jnp.transpose(w1t_v[...].astype(F32))
            w2c[...] = jnp.transpose(w2_v[...].astype(F32))

            pa = jnp.zeros((8, R), F32)
            pm = jnp.zeros((8, R), F32)
            state = {}
            for i in range(NJ):
                c0, nc, g0, ng, r0, nr = jbs[i]
                in_copy(i).wait()
                cs = pl.ds(c0, nc)
                if c0 in state:
                    s, m, cnt = state[c0]
                else:
                    s, m, cnt = jnp.zeros((nc, W), F32), jnp.full((nc, W), -jnp.inf, F32), 0
                nrows = ng * nr
                if nrows <= 32 and nc == 8:
                    vs = [xbuf[g, r, cs, :].astype(F32) for g in range(g0, g0 + ng) for r in range(r0, r0 + nr)]
                    ss, ms = list(vs), list(vs)
                    while len(ss) > 1:
                        ss = [ss[k] + ss[k + 1] if k + 1 < len(ss) else ss[k] for k in range(0, len(ss), 2)]
                        ms = [jnp.maximum(ms[k], ms[k + 1]) if k + 1 < len(ms) else ms[k] for k in range(0, len(ms), 2)]
                    s = s + ss[0]
                    m = jnp.maximum(m, ms[0])
                else:
                    U = unroll1 * (4 if nc <= 8 else (2 if nc <= 16 else 1))
                    assert nr % U == 0
                    nU = nr // U
                    def body(t, carry):
                        s, m = carry
                        g = g0 + t // nU
                        r = r0 + (t % nU) * U
                        vs = [xbuf[g, r + u, cs, :].astype(F32) for u in range(U)]
                        if nc <= 8:
                            ss, ms = list(vs), list(vs)
                            while len(ss) > 1:
                                ss = [ss[k] + ss[k + 1] for k in range(0, len(ss), 2)]
                                ms = [jnp.maximum(ms[k], ms[k + 1]) for k in range(0, len(ms), 2)]
                            return s + ss[0], jnp.maximum(m, ms[0])
                        for v in vs:
                            s = s + v
                            m = jnp.maximum(m, v)
                        return s, m
                    s, m = lax.fori_loop(0, ng * nU, body, (s, m))
                cnt += nrows
                state[c0] = (s, m, cnt)
                if cnt == H:
                    gap = _rnd(jnp.sum(s, axis=1, keepdims=True) * inv_hw)
                    gmp = jnp.max(m, axis=1, keepdims=True)
                    wblk = w1c[cs, :]
                    ta = gap * wblk
                    tm = gmp * wblk
                    for k in range(nc // 8):
                        pa = pa + ta[8 * k:8 * k + 8]
                        pm = pm + tm[8 * k:8 * k + 8]
            ha = jnp.maximum(_rnd(jnp.sum(pa, axis=0, keepdims=True)), 0.0)
            hm = jnp.maximum(_rnd(jnp.sum(pm, axis=0, keepdims=True)), 0.0)

            def scale_for(c0, nc):
                wb = w2c[pl.ds(c0, nc), :]
                za = _rnd(jnp.sum(ha * wb, axis=1, keepdims=True))
                zm = _rnd(jnp.sum(hm * wb, axis=1, keepdims=True))
                z = _rnd(za + zm)
                return _rnd(jax.nn.sigmoid(z))

            def out_copy(g0, ng, hr, c0, nc):
                sl = (pl.ds(g0, ng), hr, pl.ds(c0, nc))
                return pltpu.make_async_copy(xbuf.at[sl], o_hbm.at[sl], out_sem.at[0])

            def scale_rows(g, hr, cs, sv):
                xbuf[g, hr, cs, :] = (xbuf[g, hr, cs, :].astype(F32) * sv).astype(BF16)

            for cb in range(NCB):
                cs = pl.ds(cb * CB, CB)
                sv = jnp.broadcast_to(scale_for(cb * CB, CB), (CB, W))
                scl[cs, :] = sv
                if cb == 0 and split_first:
                    for g in range(G):
                        scale_rows(g, 0, cs, sv)
                        out_copy(g, 1, 0, 0, CB).start()
                else:
                    for g in range(G):
                        scale_rows(g, 0, cs, sv)
                    out_copy(0, G, 0, cb * CB, CB).start()

            def body2(hr, carry):
                for cb in range(NCB):
                    cs = pl.ds(cb * CB, CB)
                    sv = scl[cs, :]
                    for g in range(G):
                        scale_rows(g, hr, cs, sv)
                    out_copy(0, G, hr, cb * CB, CB).start()
                return carry
            lax.fori_loop(1, Sh, body2, 0)
            pltpu.make_async_copy(xbuf, o_hbm, out_sem.at[0]).wait()

        out = pl.pallas_call(
            kernel,
            out_shape=jax.ShapeDtypeStruct((G, Sh, C, W), x.dtype),
            in_specs=[pl.BlockSpec(memory_space=pl.ANY)] * 3,
            out_specs=pl.BlockSpec(memory_space=pl.ANY),
            scratch_shapes=[
                pltpu.VMEM((G, Sh, C, W), x.dtype),
                pltpu.VMEM((R, C), w1.dtype),
                pltpu.VMEM((R, C), w2.dtype),
                pltpu.VMEM((C, R), F32),
                pltpu.VMEM((C, R), F32),
                pltpu.VMEM((C, W), F32),
                pltpu.SemaphoreType.DMA((NJ,)),
                pltpu.SemaphoreType.DMA((2,)),
                pltpu.SemaphoreType.DMA((1,)),
            ],
            compiler_params=pltpu.CompilerParams(vmem_limit_bytes=64 * 1024 * 1024, disable_semaphore_checks=nocheck),
        )(xt, w1t, w2)
        return jnp.transpose(out.reshape(B, H, C, W), (0, 1, 3, 2))
    return fn


_impl = make(split_first=False)


@jax.jit
def pallas_standalone__channel_attn_cbam__vision_kernel(x: jax.Array, w1: jax.Array, w2: jax.Array):
    return _impl(x, w1, w2)
```

```python
import functools
import jax, jax.numpy as jnp
from jax import lax
import jax.experimental.pallas as pl
import jax.experimental.pallas.tpu as pltpu

F32 = jnp.float32
BF16 = jnp.bfloat16

def _rnd(v):
    return v.astype(BF16).astype(F32)

def _tree(vs, op):
    vs = list(vs)
    while len(vs) > 1:
        vs = [op(vs[k], vs[k + 1]) if k + 1 < len(vs) else vs[k] for k in range(0, len(vs), 2)]
    return vs[0]

TAIL = [(0, 64, 0, 32), (64, 64, 0, 32), (128, 32, 0, 32), (160, 16, 0, 32), (176, 8, 0, 32), (184, 8, 0, 24), (184, 8, 24, 8)]

def make(tail=TAIL, Sh=32, CB=32, AB=32, U=8, nocheck=True, nobounds=False, splitA=(16, 16), barrier=True,
         cbloop=False, tanh=True):
    def fn(x, w1, w2):
        B, H, W, C = x.shape
        R = w1.shape[1]
        assert B == 1
        G = H // Sh
        NCB = C // CB
        NAB = C // AB
        xt = jnp.transpose(x, (0, 1, 3, 2)).reshape(G, Sh, C, W)
        w1t = jnp.transpose(w1)
        NB = G - 1
        NT = len(tail)
        inv_hw = 1.0 / (H * W)

        def kernel(x_hbm, w1t_hbm, w2_hbm, o_hbm, xbuf, w1t_v, w2_v, w1c, w2c, scl, sacc, macc, dummy,
                   in_sems, w_sem, out_sem):
            def bulk_copy(g):
                return pltpu.make_async_copy(x_hbm.at[g], xbuf.at[g], in_sems.at[g])
            def tail_copy(i):
                c0, nc, r0, nr = tail[i]
                sl = (G - 1, pl.ds(r0, nr), pl.ds(c0, nc))
                return pltpu.make_async_copy(x_hbm.at[sl], xbuf.at[sl], in_sems.at[NB + i])
            wc1 = pltpu.make_async_copy(w1t_hbm, w1t_v, w_sem.at[0])
            wc2 = pltpu.make_async_copy(w2_hbm, w2_v, w_sem.at[1])
            for g in range(NB):
                bulk_copy(g).start(priority=1)
            for i in range(NT):
                tail_copy(i).start(priority=1)
            wc1.start()
            wc2.start()
            sacc[...] = jnp.zeros(sacc.shape, F32)
            macc[...] = jnp.full(macc.shape, -jnp.inf, F32)
            wc1.wait()
            wc2.wait()
            if barrier:
                wc3 = pltpu.make_async_copy(w2_v.at[pl.ds(0, 16)], dummy, w_sem.at[2])
                wc3.start()
            w1c[...] = jnp.transpose(w1t_v[...].astype(F32))
            w2c[...] = jnp.transpose(w2_v[...].astype(F32))

            def accum(g, r0, nr, c0, nc, s, m):
                cs = pl.ds(c0, nc)
                nv = nc // 8
                u = min(nr, max(1, U * 32 // nc))
                while nr % u:
                    u -= 1
                def step(r, s, m):
                    if nv >= 2:
                        for k in range(u):
                            v = xbuf[g, r + k, cs, :].astype(F32)
                            s = s + v
                            m = jnp.maximum(m, v)
                        return s, m
                    grp = 4
                    for k0 in range(0, u, grp):
                        vs = [xbuf[g, r + k, cs, :].astype(F32) for k in range(k0, min(u, k0 + grp))]
                        s = s + _tree(vs, jnp.add)
                        m = jnp.maximum(m, _tree(vs, jnp.maximum))
                    return s, m
                if u == nr:
                    return step(r0, s, m)
                def body(t, carry):
                    return step(r0 + t * u, *carry)
                return lax.fori_loop(0, nr // u, body, (s, m))

            def bulk_body(g, carry):
                bulk_copy(g).wait()
                def ab_body(ab, carry2):
                    c0 = pl.multiple_of(ab * AB, AB)
                    cs = pl.ds(c0, AB)
                    s, m = accum(g, 0, Sh, c0, AB, sacc[cs, :], macc[cs, :])
                    sacc[cs, :] = s
                    macc[cs, :] = m
                    return carry2
                return lax.fori_loop(0, NAB, ab_body, carry)
            lax.fori_loop(0, NB, bulk_body, 0)

            def finalize(c0, nc, s, m, pa, pm):
                cs = pl.ds(c0, nc)
                gap = _rnd(jnp.sum(s, axis=1, keepdims=True) * inv_hw)
                gmp = jnp.max(m, axis=1, keepdims=True)
                wblk = w1c[cs, :]
                ta = gap * wblk
                tm = gmp * wblk
                for k in range(nc // 8):
                    pa = pa + ta[8 * k:8 * k + 8]
                    pm = pm + tm[8 * k:8 * k + 8]
                return pa, pm

            pa = jnp.zeros((8, R), F32)
            pm = jnp.zeros((8, R), F32)
            state = {}
            for i in range(NT):
                c0, nc, r0, nr = tail[i]
                tail_copy(i).wait()
                if nc > AB:
                    assert nc % AB == 0 and nr == Sh
                    def tb(k, carry):
                        cc = pl.multiple_of(c0 + k * AB, AB)
                        cs = pl.ds(cc, AB)
                        s, m = accum(G - 1, 0, Sh, cc, AB, sacc[cs, :], macc[cs, :])
                        return finalize(cc, AB, s, m, *carry)
                    pa, pm = lax.fori_loop(0, nc // AB, tb, (pa, pm))
                    continue
                cs = pl.ds(c0, nc)
                if c0 in state:
                    s, m, cnt = state[c0]
                else:
                    s, m, cnt = sacc[cs, :], macc[cs, :], 0
                s, m = accum(G - 1, r0, nr, c0, nc, s, m)
                cnt += nr
                state[c0] = (s, m, cnt)
                if cnt == Sh:
                    pa, pm = finalize(c0, nc, s, m, pa, pm)
            ha = jnp.maximum(_rnd(jnp.sum(pa, axis=0, keepdims=True)), 0.0)
            hm = jnp.maximum(_rnd(jnp.sum(pm, axis=0, keepdims=True)), 0.0)
            hs = ha + hm

            def scale_for(c0, nc):
                wb = w2c[pl.ds(c0, nc), :]
                z = jnp.sum(hs * wb, axis=1, keepdims=True)
                if tanh:
                    sg = 0.5 * jnp.tanh(0.5 * z) + 0.5
                else:
                    sg = jax.nn.sigmoid(z)
                return _rnd(sg)

            def out_copy(hr, c0, nc):
                sl = (slice(None), hr, pl.ds(c0, nc))
                return pltpu.make_async_copy(xbuf.at[sl], o_hbm.at[sl], out_sem.at[0])

            def scale_rows(g, hr, cs, sv):
                xbuf[g, hr, cs, :] = (xbuf[g, hr, cs, :].astype(F32) * sv).astype(BF16)

            def block(hr, c0, nc, sv):
                cs = pl.ds(c0, nc)
                for g in range(G):
                    scale_rows(g, hr, cs, sv)
                out_copy(hr, c0, nc).start()

            ca = 0
            for n in splitA:
                sv = jnp.broadcast_to(scale_for(ca, n), (n, W))
                scl[pl.ds(ca, n), :] = sv
                block(0, ca, n, sv)
                ca += n
            assert ca % CB == 0
            if barrier:
                wc3.wait()
            if cbloop:
                scl[pl.ds(ca, C - ca), :] = jnp.broadcast_to(scale_for(ca, C - ca), (C - ca, W))
                def body2(t, carry):
                    hr = t // NCB
                    c0 = pl.multiple_of((t % NCB) * CB, CB)
                    block(hr, c0, CB, scl[pl.ds(c0, CB), :])
                    return carry
                lax.fori_loop(ca // CB, Sh * NCB, body2, 0)
            else:
                for cb in range(ca // CB, NCB):
                    sv = jnp.broadcast_to(scale_for(cb * CB, CB), (CB, W))
                    scl[pl.ds(cb * CB, CB), :] = sv
                    block(0, cb * CB, CB, sv)
                def body2(hr, carry):
                    for cb in range(NCB):
                        block(hr, cb * CB, CB, scl[pl.ds(cb * CB, CB), :])
                    return carry
                lax.fori_loop(1, Sh, body2, 0)
            pltpu.make_async_copy(xbuf, o_hbm, out_sem.at[0]).wait()

        out = pl.pallas_call(
            kernel,
            out_shape=jax.ShapeDtypeStruct((G, Sh, C, W), x.dtype),
            in_specs=[pl.BlockSpec(memory_space=pl.ANY)] * 3,
            out_specs=pl.BlockSpec(memory_space=pl.ANY),
            scratch_shapes=[
                pltpu.VMEM((G, Sh, C, W), x.dtype),
                pltpu.VMEM((R, C), w1.dtype),
                pltpu.VMEM((R, C), w2.dtype),
                pltpu.VMEM((C, R), F32),
                pltpu.VMEM((C, R), F32),
                pltpu.VMEM((C, W), F32),
                pltpu.VMEM((C, W), F32),
                pltpu.VMEM((C, W), F32),
                pltpu.VMEM((16, C), w2.dtype),
                pltpu.SemaphoreType.DMA((NB + NT,)),
                pltpu.SemaphoreType.DMA((3,)),
                pltpu.SemaphoreType.DMA((1,)),
            ],
            compiler_params=pltpu.CompilerParams(vmem_limit_bytes=64 * 1024 * 1024, disable_semaphore_checks=nocheck,
                                                 disable_bounds_checks=nobounds),
        )(xt, w1t, w2)
        return jnp.transpose(out.reshape(B, H, C, W), (0, 1, 3, 2))
    return fn


_impl = make()


@jax.jit
def pallas_standalone__channel_attn_cbam__vision_kernel(x: jax.Array, w1: jax.Array, w2: jax.Array):
    return _impl(x, w1, w2)
```

```python
import jax
import jax.numpy as jnp
from jax import lax
import jax.experimental.pallas as pl
import jax.experimental.pallas.tpu as pltpu

F32 = jnp.float32
BF16 = jnp.bfloat16

_SH = 32
_CB = 32
_AB = 32
_JB = 16
_U = 8
_FIRST = (16, 16)


def _rnd(v):
    return v.astype(BF16).astype(F32)


def _tree(vs, op):
    vs = list(vs)
    while len(vs) > 1:
        vs = [op(vs[k], vs[k + 1]) if k + 1 < len(vs) else vs[k] for k in range(0, len(vs), 2)]
    return vs[0]


def _tail_jobs(c, sh):
    cm = c - 16
    return [
        (0, cm, 0, sh // 2),
        (0, cm, sh // 2, sh // 4),
        (0, c // 2, 3 * sh // 4, sh // 4),
        (c // 2, c // 4, 3 * sh // 4, sh // 4),
        (3 * c // 4, cm - 3 * c // 4, 3 * sh // 4, sh // 4),
        (cm, 8, 0, sh),
        (cm + 8, 8, 0, 3 * sh // 4),
        (cm + 8, 8, 3 * sh // 4, sh // 4),
    ]


def _compiler_params():
    vmem = 64 * 1024 * 1024
    try:
        return pltpu.CompilerParams(vmem_limit_bytes=vmem, disable_semaphore_checks=True)
    except TypeError:
        return pltpu.CompilerParams(vmem_limit_bytes=vmem)


@jax.jit
def pallas_standalone__channel_attn_cbam__vision_kernel(
    x: jax.Array,
    w1: jax.Array,
    w2: jax.Array,
):
    B, H, W, C = x.shape
    R = w1.shape[1]
    SH, CB, AB, JB, U = _SH, _CB, _AB, _JB, _U
    assert B == 1 and H % SH == 0 and C % CB == 0 and C % AB == 0 and sum(_FIRST) % CB == 0
    G = H // SH
    NCB = C // CB
    NAB = C // AB
    NB = G - 1
    jobs = _tail_jobs(C, SH)
    NT = len(jobs)
    inv_hw = 1.0 / (H * W)

    xt = jnp.transpose(x, (0, 1, 3, 2)).reshape(G, SH, C, W)
    w1t = jnp.transpose(w1)

    def kernel(x_hbm, w1t_hbm, w2_hbm, o_hbm,
               xbuf, w1t_v, w2_v, w1c, w2c, scl, sacc, macc, fence_buf,
               in_sems, w_sems):
        out_sem = in_sems.at[0]

        def bulk_copy(g):
            return pltpu.make_async_copy(x_hbm.at[g], xbuf.at[g], in_sems.at[g])

        def tail_copy(i):
            c0, nc, r0, nr = jobs[i]
            sl = (G - 1, pl.ds(r0, nr), pl.ds(c0, nc))
            return pltpu.make_async_copy(x_hbm.at[sl], xbuf.at[sl], in_sems.at[NB + i])

        w1_copy = pltpu.make_async_copy(w1t_hbm, w1t_v, w_sems.at[0])
        w2_copy = pltpu.make_async_copy(w2_hbm, w2_v, w_sems.at[1])
        for g in range(NB):
            bulk_copy(g).start(priority=1)
        for i in range(NT):
            tail_copy(i).start(priority=1)
        w1_copy.start()
        w2_copy.start()
        sacc[...] = jnp.zeros(sacc.shape, F32)
        macc[...] = jnp.full(macc.shape, -jnp.inf, F32)
        w1_copy.wait()
        w2_copy.wait()
        fence = pltpu.make_async_copy(w2_v.at[pl.ds(0, 16)], fence_buf, w_sems.at[0])
        fence.start()
        w1c[...] = jnp.transpose(w1t_v[...].astype(F32))
        w2c[...] = jnp.transpose(w2_v[...].astype(F32))

        def accum(g, r0, nr, c0, nc, s, m):
            cs = pl.ds(c0, nc)
            u = min(nr, max(1, U * AB // nc))
            while nr % u:
                u -= 1

            def step(r, s, m):
                if nc > 8:
                    for k in range(u):
                        v = xbuf[g, r + k, cs, :].astype(F32)
                        s = s + v
                        m = jnp.maximum(m, v)
                    return s, m
                for k0 in range(0, u, 4):
                    vs = [xbuf[g, r + k, cs, :].astype(F32) for k in range(k0, min(u, k0 + 4))]
                    s = s + _tree(vs, jnp.add)
                    m = jnp.maximum(m, _tree(vs, jnp.maximum))
                return s, m

            if u == nr:
                return step(r0, s, m)
            return lax.fori_loop(0, nr // u, lambda t, c: step(r0 + t * u, *c), (s, m))

        def accum_blocks(g, r0, nr, cbase, nblk, blk):
            def body(ab, carry):
                c0 = pl.multiple_of(cbase + ab * blk, 8)
                cs = pl.ds(c0, blk)
                s, m = accum(g, r0, nr, c0, blk, sacc[cs, :], macc[cs, :])
                sacc[cs, :] = s
                macc[cs, :] = m
                return carry
            lax.fori_loop(0, nblk, body, 0)

        def bulk_body(g, carry):
            bulk_copy(g).wait()
            accum_blocks(g, 0, SH, 0, NAB, AB)
            return carry
        lax.fori_loop(0, NB, bulk_body, 0)

        def finalize(c0, nc, s, m, pa, pm):
            gap = _rnd(jnp.sum(s, axis=1, keepdims=True) * inv_hw)
            gmp = jnp.max(m, axis=1, keepdims=True)
            wblk = w1c[pl.ds(c0, nc), :]
            ta = gap * wblk
            tm = gmp * wblk
            for k in range(nc // 8):
                pa = pa + ta[8 * k:8 * k + 8]
                pm = pm + tm[8 * k:8 * k + 8]
            return pa, pm

        pa = jnp.zeros((8, R), F32)
        pm = jnp.zeros((8, R), F32)
        rows_done = [0] * (C // 8)
        live = {}
        for i in range(NT):
            c0, nc, r0, nr = jobs[i]
            tail_copy(i).wait()
            blocks = range(c0 // 8, (c0 + nc) // 8)
            done = all(rows_done[k] + nr == SH for k in blocks)
            for k in blocks:
                rows_done[k] += nr
            if not done and nc > AB:
                assert nc % JB == 0
                accum_blocks(G - 1, r0, nr, c0, nc // JB, JB)
                continue
            for cc in range(c0, c0 + nc, AB):
                ncc = min(AB, c0 + nc - cc)
                if cc in live:
                    n_live, s, m = live.pop(cc)
                    assert n_live == ncc
                else:
                    s, m = sacc[pl.ds(cc, ncc), :], macc[pl.ds(cc, ncc), :]
                s, m = accum(G - 1, r0, nr, cc, ncc, s, m)
                if done:
                    pa, pm = finalize(cc, ncc, s, m, pa, pm)
                else:
                    live[cc] = (ncc, s, m)
        assert all(r == SH for r in rows_done) and not live

        ha = _rnd(jnp.sum(pa, axis=0, keepdims=True))
        hm = _rnd(jnp.sum(pm, axis=0, keepdims=True))
        ha = ha * (ha > 0).astype(F32)
        hm = hm * (hm > 0).astype(F32)

        def scale_for(c0, nc):
            wb = w2c[pl.ds(c0, nc), :]
            za = _rnd(jnp.sum(ha * wb, axis=1, keepdims=True))
            zm = _rnd(jnp.sum(hm * wb, axis=1, keepdims=True))
            sg = _rnd(jax.nn.sigmoid(_rnd(za + zm)))
            sv = jnp.broadcast_to(sg, (nc, W))
            scl[pl.ds(c0, nc), :] = sv
            return sv

        def emit(hr, c0, nc, sv):
            cs = pl.ds(c0, nc)
            for g in range(G):
                xbuf[g, hr, cs, :] = (xbuf[g, hr, cs, :].astype(F32) * sv).astype(BF16)
            sl = (slice(None), hr, cs)
            pltpu.make_async_copy(xbuf.at[sl], o_hbm.at[sl], out_sem).start()

        ca = 0
        for n in _FIRST:
            emit(0, ca, n, scale_for(ca, n))
            ca += n
        fence.wait()
        for cb in range(ca // CB, NCB):
            emit(0, cb * CB, CB, scale_for(cb * CB, CB))

        def row_body(hr, carry):
            for cb in range(NCB):
                emit(hr, cb * CB, CB, scl[pl.ds(cb * CB, CB), :])
            return carry
        lax.fori_loop(1, SH, row_body, 0)

        pltpu.make_async_copy(xbuf, o_hbm, out_sem).wait()

    out = pl.pallas_call(
        kernel,
        out_shape=jax.ShapeDtypeStruct((G, SH, C, W), x.dtype),
        in_specs=[pl.BlockSpec(memory_space=pl.ANY)] * 3,
        out_specs=pl.BlockSpec(memory_space=pl.ANY),
        scratch_shapes=[
            pltpu.VMEM((G, SH, C, W), x.dtype),
            pltpu.VMEM((R, C), w1.dtype),
            pltpu.VMEM((R, C), w2.dtype),
            pltpu.VMEM((C, R), F32),
            pltpu.VMEM((C, R), F32),
            pltpu.VMEM((C, W), F32),
            pltpu.VMEM((C, W), F32),
            pltpu.VMEM((C, W), F32),
            pltpu.VMEM((16, C), w2.dtype),
            pltpu.SemaphoreType.DMA((NB + NT,)),
            pltpu.SemaphoreType.DMA((2,)),
        ],
        compiler_params=_compiler_params(),
    )(xt, w1t, w2)
    return jnp.transpose(out.reshape(B, H, C, W), (0, 1, 3, 2))
```
